```python
import os as _os
_os.environ.setdefault('JAX_PLATFORMS', 'cpu')
import jax
import jax.numpy as jnp

def _softmax(x, axis=-1):
    return jax.nn.softmax(x, axis=axis)

def _gelu(x):
    return jax.nn.gelu(x, approximate=True)

def _silu(x):
    return jax.nn.silu(x)

def _sigmoid(x):
    return jax.nn.sigmoid(x)

def _layernorm(x, axis=-1, eps=1e-05):
    m = jnp.mean(x, axis=axis, keepdims=True)
    v = jnp.var(x, axis=axis, keepdims=True)
    return (x - m) / jnp.sqrt(v + eps)

def _scatter_add(tgt, idx, src, axis=0):
    return tgt.at[idx].add(src)

def _segment_sum(src, seg, n):
    return jax.ops.segment_sum(src, seg, n)

class _Rng:

    def __init__(self, key):
        self._k = key

    def _next(self):
        self._k, sub = jax.random.split(self._k)
        return sub

    def normal(self, shape):
        return jax.random.normal(self._next(), shape, dtype=jnp.bfloat16)

    def randint(self, lo, hi, shape):
        return jax.random.randint(self._next(), shape, lo, hi, dtype=jnp.int32)

    def uniform(self, shape, lo=0.0, hi=1.0):
        return jax.random.uniform(self._next(), shape, jnp.bfloat16, lo, hi)

    def permutation(self, n):
        return jax.random.permutation(self._next(), n)
kernel_name = 'interleave_layers__memory_aug_recurrent_mem_tr__mixer_token_mlp__prompt'

def setup_inputs():
    _rng = _Rng(jax.random.key(int.from_bytes(__import__("os").urandom(4), "little")))
    _w = lambda a: (lambda t: t.astype(jnp.bfloat16) if jnp.issubdtype(t.dtype, jnp.floating) else t)(jnp.asarray(a))

    def _A_setup():
        B, S, Dm = (1, 2048, 640)
        H, Dh = (32, 128)
        M, seg = (8, 32)
        seg = min(seg, S)
        S = S // seg * seg
        return {'x': _w((lambda *s: _rng.normal(s) * 0.05)(B, S, Dm)), 'mem0': _w((lambda *s: _rng.normal(s) * 0.2)(B, M, Dm)), 'Wq': _w((lambda *s: _rng.normal(s) * 0.8)(Dm, H, Dh) * Dm ** (-0.5)), 'Wk': _w((lambda *s: _rng.normal(s) * 0.8)(Dm, H, Dh) * Dm ** (-0.5)), 'Wv': _w((lambda *s: _rng.normal(s) * 0.2)(Dm, H, Dh) * Dm ** (-0.5)), 'Wo': _w((lambda *s: _rng.normal(s) * 0.2)(H, Dh, Dm) * (H * Dh) ** (-0.5)), 'seg_len': seg}
    _A_in = _A_setup()

    def _B_setup():
        B, S, D, F = (1, 2048, 640, 1728)
        return {'x': _w((lambda *s: _rng.normal(s) * 0.05)(B, S, D)), 'w1': _w((lambda *s: _rng.normal(s) * 0.2)(S, F) * S ** (-0.5)), 'b1': _w((lambda *s: _rng.normal(s) * 0.2)(F) * 0.02), 'w2': _w((lambda *s: _rng.normal(s) * 0.2)(F, S) * F ** (-0.5)), 'b2': _w((lambda *s: _rng.normal(s) * 0.2)(S) * 0.02)}
    _B_in = _B_setup()
    return {'A_x': _A_in['x'], 'A_mem0': _A_in['mem0'], 'A_Wq': _A_in['Wq'], 'A_Wk': _A_in['Wk'], 'A_Wv': _A_in['Wv'], 'A_Wo': _A_in['Wo'], 'A_seg_len': _A_in['seg_len'], 'B_x': _B_in['x'], 'B_w1': _B_in['w1'], 'B_b1': _B_in['b1'], 'B_w2': _B_in['w2'], 'B_b2': _B_in['b2']}

def reference(A_x, A_mem0, A_Wq, A_Wk, A_Wv, A_Wo, A_seg_len, B_x, B_w1, B_b1, B_w2, B_b2):

    def _A_ref(x, mem0, Wq, Wk, Wv, Wo, seg_len):
        B, S, Dm = x.shape
        H, Dh = (Wq.shape[1], Wq.shape[2])
        M = mem0.shape[1]
        scale = Dh ** (-0.5)
        n_seg = S // seg_len
        L = M + seg_len
        idx = jnp.arange(L)
        mask = (idx[:, None] < M) | (idx[:, None] >= idx[None, :])
        mem = mem0
        outs = []
        for s in range(n_seg):
            xs = x[:, s * seg_len:(s + 1) * seg_len, :].copy()
            h = jnp.concatenate([mem, xs], axis=1)
            q = jnp.einsum('btd,dhe->bhte', h, Wq)
            k = jnp.einsum('btd,dhe->bhte', h, Wk)
            v = jnp.einsum('btd,dhe->bhte', h, Wv)
            scores = jnp.einsum('bhqe,bhke->bhqk', q, k) * scale
            scores = jnp.where(mask[None, None], scores, -1000000000.0)
            p = _softmax(scores, axis=-1)
            o = jnp.einsum('bhqk,bhke->bhqe', p, v)
            o = jnp.einsum('bhte,hed->btd', o, Wo)
            mem = o[:, :M, :].copy()
            outs.append(o[:, M:, :])
        return jnp.concatenate(outs, axis=1)

    def _B_ref(x, w1, b1, w2, b2):
        B, S, D = x.shape
        h = _layernorm(x, axis=-1)
        u = jnp.einsum('bsd,sf->bdf', h, w1) + b1
        u = _gelu(u)
        y = jnp.einsum('bdf,fs->bds', u, w2) + b2
        return (lambda x, *d: x.transpose(*d))(y, 0, 2, 1)
    x = A_x
    x = x + _A_ref(_layernorm(x, axis=-1), A_mem0, A_Wq, A_Wk, A_Wv, A_Wo, A_seg_len)
    x = x + _B_ref(_layernorm(x, axis=-1), B_w1, B_b1, B_w2, B_b2)
    x = x + _A_ref(_layernorm(x, axis=-1), A_mem0, A_Wq, A_Wk, A_Wv, A_Wo, A_seg_len)
    x = x + _B_ref(_layernorm(x, axis=-1), B_w1, B_b1, B_w2, B_b2)
    return x
```

```python
import functools

import jax
import jax.numpy as jnp
import numpy as np
from jax import lax
from jax.experimental import pallas as pl
from jax.experimental.pallas import tpu as pltpu

_F32, _BF16, _U32 = jnp.float32, jnp.bfloat16, jnp.uint32
_NT = (((1,), (1,)), ((), ()))
_TN = (((0,), (0,)), ((), ()))
_LANES = 128


def _layernorm(x):
    m = jnp.mean(x, axis=-1, keepdims=True)
    d = x - m
    v = jnp.mean(d * d, axis=-1, keepdims=True)
    return d * lax.rsqrt(v + 1e-5)


def _gelu(x):
    c = float(np.sqrt(2.0 / np.pi))
    return 0.5 * x * (1.0 + jnp.tanh(c * (x + 0.044715 * (x * x * x))))


def _kernel(x_hbm, mem0_ref, wq_hbm, wk_hbm, wv_hbm, wo_hbm, w1_hbm, b1_ref, w2_hbm, b2_ref,
            out_hbm,
            xio_ref, xres_ref, hb_ref, raw_ref, wqkv_ref, wo_raw_ref, wo_ref, w1_ref, w2_ref,
            b1c_ref, b2c_ref, g_ref, sems, *, seg):
    S, D = x_hbm.shape
    _, H, E = wq_hbm.shape
    M = mem0_ref.shape[0]
    F = w1_hbm.shape[0]
    L = seg + M
    n_seg = S // seg
    n_kt = D // _LANES

    x_cp = pltpu.make_async_copy(x_hbm, xio_ref, sems.at[0])
    wo_cp = pltpu.make_async_copy(wo_hbm, wo_raw_ref, sems.at[1])
    w1_cp = pltpu.make_async_copy(w1_hbm, w1_ref, sems.at[2])
    w2_cp = pltpu.make_async_copy(w2_hbm, w2_ref, sems.at[3])
    raw_cps = [
        [pltpu.make_async_copy(w.at[pl.ds(j * _LANES, _LANES)],
                               raw_ref.at[i, pl.ds(j * _LANES, _LANES)],
                               sems.at[4 + i * n_kt + j]) for j in range(n_kt)]
        for i, w in enumerate((wq_hbm, wk_hbm, wv_hbm))]
    x_cp.start()
    for cps in raw_cps:
        for cp in cps:
            cp.start()
    wo_cp.start()
    w1_cp.start()
    w2_cp.start()

    def bias_column(b_ref, dst_ref):
        n = b_ref.shape[0]
        row = b_ref[...].astype(_F32).reshape(1, n)
        for c0 in range(0, n, _LANES):
            c1 = min(n, c0 + _LANES)
            dst_ref[c0:c1, :] = jnp.broadcast_to(row[:, c0:c1], (_LANES, c1 - c0)).T

    bias_column(b1_ref, b1c_ref)
    bias_column(b2_ref, b2c_ref)

    x_cp.wait()

    @pl.loop(0, S // 128)
    def _(i):
        rows = pl.ds(pl.multiple_of(i * 128, 128), 128)
        xres_ref[rows, :] = xio_ref[rows, :].astype(_F32)

    for i in range(3):
        for j in range(n_kt):
            raw_cps[i][j].wait()

            @pl.loop(j * (_LANES // 16), (j + 1) * (_LANES // 16))
            def _(t, i=i):
                blk = raw_ref[i, pl.ds(pl.multiple_of(t * 16, 16), 16)]
                wqkv_ref[:, pl.ds(pl.multiple_of(t * 8, 8), 8), i * E:(i + 1) * E] = (
                    pltpu.bitcast(jnp.swapaxes(blk, 0, 1), _U32))

    wo_cp.wait()

    @pl.loop(0, H)
    def _(h):
        wo_ref[pl.ds(pl.multiple_of(h * (E // 2), E // 2), E // 2), :] = pltpu.bitcast(
            wo_raw_ref[pl.ds(pl.multiple_of(h * E, E), E), :], _U32)

    scale = E ** -0.5

    def seg_rows(s):
        return pl.ds(pl.multiple_of(s * seg, seg), seg)

    def attention_step(s, mem, hx):
        ri = lax.broadcasted_iota(jnp.int32, (L, L), 0)
        ci = lax.broadcasted_iota(jnp.int32, (L, L), 1)
        mask = (ri >= seg) | (ci >= seg) | (ri >= ci)

        def scores(qkv):
            q, k, v = qkv[:, :E], qkv[:, E:2 * E], qkv[:, 2 * E:]
            sc = lax.dot_general(q, k.astype(_BF16), _NT, preferred_element_type=_F32)
            return sc, v.astype(_BF16)

        def attend(sc, v):
            sc = jnp.where(mask, sc * scale, -1e9)
            e = jnp.exp(sc - jnp.max(sc, axis=-1, keepdims=True))
            den = jnp.sum(e, axis=-1, keepdims=True)
            o = jnp.dot(e, v, preferred_element_type=_F32) * pltpu.reciprocal(den)
            return jnp.concatenate([o[seg:], o[:seg]], axis=0)

        def project(h0, h1):
            lhs = jnp.concatenate([outs[i] for i in range(h0, h1)], axis=1)
            w = pltpu.bitcast(wo_ref[h0 * E // 2:h1 * E // 2, :], _BF16)
            return jnp.dot(lhs, w, preferred_element_type=_F32)

        d1, d2, oc = 2, 2, 4
        h = jnp.concatenate([hx, mem], axis=0)
        qkvs, scs, outs, parts = {}, {}, {}, []
        for t in range(H + d1 + d2):
            if t < H:
                qkvs[t] = jnp.dot(h, pltpu.bitcast(wqkv_ref[t], _BF16),
                                  preferred_element_type=_F32)
            else:
                parts.append(project((t - H) * oc, (t - H + 1) * oc))
            if 0 <= t - d1 < H:
                scs[t - d1] = scores(qkvs.pop(t - d1))
            if 0 <= t - d1 - d2 < H:
                outs[t - d1 - d2] = attend(*scs.pop(t - d1 - d2))
        parts.append(project((d1 + d2) * oc, H))
        out = functools.reduce(lambda a, b: a + b, parts)
        xres_ref[seg_rows(s), :] += out[M:]
        return out[:M]

    def mixer_input(s):
        hb_ref[seg_rows(s), :] = _layernorm(_layernorm(xres_ref[seg_rows(s), :])).astype(_BF16)

    def attention_layer():
        unroll = 2

        def body(i, carry):
            mem, hx = carry
            for u in range(unroll):
                s = i * unroll + u
                mixer_input(jnp.maximum(s - 1, 0))
                hx_next = _layernorm(xres_ref[seg_rows(jnp.minimum(s + 1, n_seg - 1)), :])
                mem = attention_step(s, mem, hx)
                hx = hx_next
            return mem, hx

        lax.fori_loop(0, n_seg // unroll, body,
                      (mem0_ref[...].astype(_F32), _layernorm(xres_ref[0:seg, :])))
        mixer_input(n_seg - 1)

    chunk = 512

    def out_copy(c):
        rows = pl.ds(c * chunk, chunk)
        return pltpu.make_async_copy(xio_ref.at[rows], out_hbm.at[rows], sems.at[c])

    def mixer_layer(layer):
        for n0 in range(0, F, chunk):
            n1 = min(F, n0 + chunk)
            u = jnp.dot(w1_ref[n0:n1, :], hb_ref[...], preferred_element_type=_F32)
            u = u + jnp.tile(b1c_ref[n0:n1, :], (1, n_kt))
            g_ref[n0:n1, :] = _gelu(u).astype(_BF16)
        for c in range(S // chunk):
            rows = slice(c * chunk, (c + 1) * chunk)
            y = lax.dot_general(w2_ref[:, rows], g_ref[...], _TN, preferred_element_type=_F32)
            xn = xres_ref[rows, :] + (y + jnp.tile(b2c_ref[rows, :], (1, n_kt)))
            xres_ref[rows, :] = xn
            xio_ref[rows, :] = xn.astype(_BF16)

            @pl.when(layer == 1)
            def _(c=c):
                out_copy(c).start()

    @pl.loop(0, 2)
    def _(layer):
        attention_layer()

        @pl.when(layer == 0)
        def _():
            w1_cp.wait()
            w2_cp.wait()

        mixer_layer(layer)

    for c in range(S // chunk):
        out_copy(c).wait()


@functools.partial(jax.jit, static_argnames=("A_seg_len",))
def pallas_interleave_layers__memory_aug_recurrent_mem_tr__mixer_token_mlp__prompt_kernel(
    A_x: jax.Array,
    A_mem0: jax.Array,
    A_Wq: jax.Array,
    A_Wk: jax.Array,
    A_Wv: jax.Array,
    A_Wo: jax.Array,
    A_seg_len: int,
    B_x: jax.Array,
    B_w1: jax.Array,
    B_b1: jax.Array,
    B_w2: jax.Array,
    B_b2: jax.Array,
):
    del B_x
    _, S, D = A_x.shape
    _, H, E = A_Wq.shape
    M = A_mem0.shape[1]
    F = B_w1.shape[1]
    hbm = pl.BlockSpec(memory_space=pl.ANY)
    vmem = pl.BlockSpec(memory_space=pltpu.VMEM)
    out = pl.pallas_call(
        functools.partial(_kernel, seg=int(A_seg_len)),
        out_shape=jax.ShapeDtypeStruct((S, D), A_x.dtype),
        in_specs=[hbm, vmem, hbm, hbm, hbm, hbm, hbm, vmem, hbm, vmem],
        out_specs=hbm,
        scratch_shapes=[
            pltpu.VMEM((S, D), _BF16),
            pltpu.VMEM((S, D), _F32),
            pltpu.VMEM((S, D), _BF16),
            pltpu.VMEM((3, D, H, E), _BF16),
            pltpu.VMEM((H, D // 2, 3 * E), _U32),
            pltpu.VMEM((H * E, D), _BF16),
            pltpu.VMEM((H * E // 2, D), _U32),
            pltpu.VMEM((F, S), _BF16),
            pltpu.VMEM((F, S), _BF16),
            pltpu.VMEM((F, _LANES), _F32),
            pltpu.VMEM((S, _LANES), _F32),
            pltpu.VMEM((F, D), _BF16),
            pltpu.SemaphoreType.DMA((4 + 3 * (D // _LANES),)),
        ],
        compiler_params=pltpu.CompilerParams(vmem_limit_bytes=120 * 1024 * 1024),
        name="rmt_mixer",
    )(A_x.reshape(S, D), A_mem0.reshape(M, D), A_Wq, A_Wk, A_Wv, A_Wo.reshape(H * E, D),
      B_w1.T, B_b1, B_w2, B_b2)
    return out.reshape(A_x.shape)
```

```python
import collections
import functools

import jax
import jax.numpy as jnp
import numpy as np
from jax import lax
from jax.experimental import pallas as pl
from jax.experimental.pallas import tpu as pltpu

_F32, _BF16, _U32 = jnp.float32, jnp.bfloat16, jnp.uint32
_T = 128
_G = 4

_U = [{(0, 0): 1, (1, 1): 1}, {(1, 0): 1, (1, 1): 1}, {(0, 0): 1}, {(1, 1): 1},
      {(0, 0): 1, (0, 1): 1}, {(1, 0): 1, (0, 0): -1}, {(0, 1): 1, (1, 1): -1}]
_V = [{(0, 0): 1, (1, 1): 1}, {(0, 0): 1}, {(0, 1): 1, (1, 1): -1}, {(1, 0): 1, (0, 0): -1},
      {(1, 1): 1}, {(0, 0): 1, (0, 1): 1}, {(1, 0): 1, (1, 1): 1}]
_W = {(0, 0): {0: 1, 6: 1, 3: 1, 4: -1}, (0, 1): {2: 1, 4: 1},
      (1, 0): {1: 1, 3: 1}, (1, 1): {0: 1, 5: 1, 2: 1, 1: -1}}
_MIRRORED = (1, 4, 5, 6)
_MU = [{5: {0: 1}, 0: {1: 1}, 6: {1: 1}, 1: {0: 1, 1: 1}},
       {3: {1: 1}, 4: {0: 1, 1: 1}, 2: {0: 1}, 1: {0: 1, 1: 1}}]
_MW = [[{6: 1, 1: 1, 0: -1}, {0: 1, 5: 1, 1: -1}], [{1: 1, 3: 1}, {2: 1, 4: 1}]]
_SHARED = 1
_VISITS = [(0, 0), (0, 1), (1, 0), (1, 1)]

_Order = collections.namedtuple(
    "_Order", "in_outer in_inner in_turn out_outer out_inner out_turn fifth "
              "score softmax attend finish eager out_chunks")
_LEADING = [
    [
        ('6105 3421', '0561 3421', '0000', '1065 3241', '6051 3421', '3000', '6755',
         5, 10, 10, (8, 11, 16, 23), False,
         '51:m02 78:m24 125:m46 138:l02 135:l25 140:m68 140:l58'),
        ('0651 3421', '5061 3421', '0002', '1056 3241', '6051 3421', '3000', '6755',
         5, 10, 10, (8, 13, 16, 23), True,
         '51:m02 80:m24 125:m46 138:l02 135:l25 140:m68 140:l58'),
        ('6051 3421', '5061 3421', '0000', '6015 3241', '6051 3421', '0002', '6755',
         5, 5, 10, (5, 11, 14, 23), True,
         '51:m02 80:m24 123:m46 138:l02 135:l25 140:m68 140:l58'),
        ('6051 3241', '5061 3421', '0000', '1065 3241', '6051 4321', '3000', '6755',
         5, 10, 10, (5, 11, 16, 23), False,
         '51:m02 80:m24 125:m46 138:l01 137:l15 140:m68 140:l58'),
    ], [
        ('5016 3421', '0651 2431', '0003', '5061 3241', '5061 3421', '0002', '6666',
         5, 5, 10, (5, 11, 17, 23), True,
         '53:m02 80:m24 125:m46 129:l01 140:l16 140:m68 140:l68'),
        ('5061 3421', '0651 2431', '0003', '5061 3241', '5061 3421', '0002', '4444',
         5, 5, 10, (5, 11, 17, 23), False,
         '50:m02 80:m24 125:m46 129:l01 135:l16 140:m68 140:l68'),
        ('5061 1423', '0615 2431', '0003', '1065 3241', '5061 3241', '0002', '6666',
         5, 5, 10, (5, 11, 17, 23), True,
         '50:m02 80:m24 126:m46 129:l01 135:l16 140:m68 140:l68'),
        ('5061 3421', '0651 2431', '0003', '5061 3241', '5061 3421', '0002', '6666',
         5, 5, 10, (5, 11, 18, 23), True,
         '50:m02 80:m24 130:m46 129:l01 135:l16 143:m68 140:l68'),
    ]]
_LAST = [
    [
        ('5061 3241', '1605 2431', '0020', '0651 3142', '5061 3421', '1001', '4554',
         5, 0, 8, (8, 14, 16, 23), True, '50:m01 80:m14 125:m46 130:l02 134:l26 140:m68 140:l68'),
        ('5061 3241', '1605 2341', '1000', '0651 3142', '6051 3421', '1001', '6666',
         4, 0, 11, (8, 14, 16, 23), True, '50:m01 80:m14 125:m46 130:l02 134:l26 140:m68 140:l68'),
        ('5061 3241', '5601 2431', '0000', '0651 3142', '5061 2431', '1001', '6666',
         4, 0, 12, (8, 14, 16, 23), True, '50:m01 80:m14 125:m46 130:l02 134:l26 140:m68 140:l68'),
        ('5061 3241', '1605 2431', '2332', '0651 3142', '6501 3421', '1001', '5555',
         5, 0, 13, (8, 14, 16, 23), True, '50:m01 80:m14 125:m46 130:l02 134:l26 140:m68 140:l68'),
    ], [
        ('5160 3421', '1605 2431', '0020', '0561 3241', '5061 3421', '1003', '4554',
         5, 0, 8, (8, 14, 16, 22), True,
         '50:m02 80:m24 125:m46 130:l02 135:l26 140:m68 140:l68'),
        ('5016 3421', '1605 2341', '1000', '0561 3241', '6051 3421', '1003', '6666',
         4, 0, 10, (6, 14, 16, 22), True,
         '50:m02 80:m24 127:m46 130:l02 135:l26 140:m68 143:l68'),
        ('5061 3124', '5601 2431', '0000', '0561 3241', '5061 2431', '1003', '6666',
         4, 0, 12, (8, 14, 16, 22), True,
         '50:m02 80:m24 125:m46 130:l03 134:l36 140:m68 140:l68'),
        ('5061 4231', '1605 2431', '2332', '0561 3241', '6501 3421', '1003', '5555',
         5, 0, 13, (8, 14, 16, 22), True,
         '50:m02 80:m24 126:m46 132:l01 135:l17 140:m68 140:l78'),
    ]]
_MIXER = [('1025436', '4250136', '4152036', '4102536'),
          ('1025436', '4250136', '4102563', '4102536')]


def _digits(text):
    return tuple(map(int, text))


def _visit_order(outer, inner, turn, p, q):
    ts = _digits(inner.split()[q])
    return {r: ts[k:] + ts[:k] for r, k in zip(_digits(outer.split()[p]), _digits(turn))}


def _layernorm(x, scale=None):
    m = jnp.mean(x, axis=-1, keepdims=True)
    d = x - m
    inv = lax.rsqrt(jnp.mean(d * d, axis=-1, keepdims=True) + 1e-5)
    return d * (inv if scale is None else inv * scale)


def _gelu_of_twice(h):
    c = float(np.sqrt(2.0 / np.pi))
    return h + h * jnp.tanh(h * (2 * c + (8 * c * 0.044715) * (h * h)))


def _dot(a, b):
    return jnp.dot(a, b, preferred_element_type=_F32)


def _dot_nt(a, b):
    return lax.dot_general(a, b, (((1,), (1,)), ((), ())), preferred_element_type=_F32)


def _lin(coef, get):
    terms = [(c, get(k)) for k, c in coef.items()]
    pos = [v for c, v in terms if c > 0 and v is not None]
    neg = [v for c, v in terms if c < 0 and v is not None]
    if not pos:
        return -functools.reduce(lax.add, neg) if neg else None
    return functools.reduce(lax.sub, neg, functools.reduce(lax.add, pos))


def _lin2(table, r, t, get):
    return _lin(table[r], lambda o: _lin(
        table[t], lambda n: get(2 * o[0] + n[0], 2 * o[1] + n[1])))


def _outer(table, r, get):
    return {n: _lin(table[r], lambda o: get(2 * o[0] + n[0], 2 * o[1] + n[1])) for n in _W}


def _mirror(r, block):
    return (block[0], 1 - block[1]) if r in _MIRRORED else block


def _weight_tiles(get):
    for r in range(7):
        outer = _outer(_V, r, get)
        for t in range(7):
            yield r * 7 + t, _lin(_V[t], lambda n: outer[_mirror(r, n)])


def _halves(p, q, r, t):
    if r == _SHARED and t == _SHARED:
        return (p,) if p == q else ()
    if r == _SHARED:
        return (p,)
    if t == _SHARED:
        return (q,)
    return (0, 1)


def _merged(visits):
    found = {}
    for p, q in visits:
        for r in _MU[p]:
            for t in _MU[q]:
                found.setdefault((r, t), []).extend(_halves(p, q, r, t))
    found = [(k, sorted(hs)) for k, hs in found.items() if hs]
    return dict(sorted(found, key=lambda kv: (-len(kv[1]), kv[0])))


def _memory_operands(p, q, get):
    cache = {}

    def cached(key, coef, term):
        if key not in cache:
            cache[key] = _lin(coef, term)
        return cache[key]

    return {(r, t): cached(
        (tuple(u), tuple(v)), v,
        lambda k2: cached((tuple(u), k2), u, lambda k1: get(2 * k1 + k2)))
        for r, u in _MU[p].items() for t, v in _MU[q].items()}


def _memory_result(p, q, prods):
    inner = {(r, _mirror(r, (0, j2))[1]): _lin(_MW[q][j2], lambda t: prods[r, t])
             for r in _MU[p] for j2 in (0, 1)}
    return [_lin(_MW[p][j // 2], lambda r: inner[r, j % 2]) for j in range(_G)]


def _inner_blocks(prods, rs):
    return {(r, _mirror(r, a), h): _lin(_W[a], lambda t: prods.get((r, t, h)))
            for h in (0, 1) for r in rs for a in _W}


def _add_blocks(inner, outer_blocks, done_visits, load):
    out = {}
    for h in (0, 1):
        for b in outer_blocks:
            for a in _W:
                i, j = 2 * b[0] + a[0], 2 * b[1] + a[1]
                coef = {r: c for r, c in _W[b].items() if inner.get((r, a, h)) is not None}
                if not coef:
                    continue
                started = any(h in _halves(p, q, r, t) for p, q in done_visits
                              for r in _W[b] if r in _MU[p]
                              for t in _W[_mirror(r, a)] if t in _MU[q])
                old = load(i, j, h) if started else None
                out[i, j, h] = _lin({-1: 1, **coef}, lambda r: old if r < 0 else inner[r, a, h])
    return out


def _interleave(*streams):
    ticks = sorted(((k + 0.5) / n, u) for u, (_, n) in enumerate(streams) for k in range(n))
    for _, u in ticks:
        next(streams[u][0])


def _cols(j, n=1):
    return slice(j * _T, (j + n) * _T)


def _aligned(start, n):
    return pl.ds(start if isinstance(start, int) else pl.multiple_of(start, 16), n)


def _shifted(ref, rows, max_rows):
    return ref.at[_aligned(rows, ref.shape[0] - max_rows)]


def _tiles(ref, start, n=1, axis=0):
    return jnp.concatenate(
        [pltpu.bitcast(ref[pl.ds(u // 2 * (_T // 2), _T // 2), _cols(u % 2)], _BF16)
         for u in range(start, start + n)], axis=axis)


def _put_rows(ref, tile, row, value):
    ref[pl.ds(tile // 2 * _T + row, value.shape[0]), _cols(tile % 2)] = value.astype(_BF16)


_CHUNKS = 4
_SLOTS = 3
_EARLY = (2, 3, 3, 1)
_N_EARLY = (3 * _EARLY[0] + _CHUNKS * (_EARLY[1] + 2 * _EARLY[2] + _EARLY[3])) // 2


def _kernel(x_hbm, mem0_hbm, wq_hbm, wk_hbm, wv_hbm, wo_hbm, w1_hbm, b1_hbm, w2_hbm, b2_hbm,
            out_hbm,
            stream, wt, w1t, w2n, tbuf, mo, fin, n5, obuf, pool, ring, cbuf, early_lhs,
            mem0_ref, mem_ref, b1_ref, b2_ref, zero_ref, sems, *, seg):
    S, D = x_hbm.shape
    H = wo_hbm.shape[0] // _T
    M = mem0_hbm.shape[0]
    F = w1_hbm.shape[0]
    L = seg + M
    NG = H // _G
    GR = _G * seg
    n_grp = S // GR
    HR = seg // 2
    n_lead = (n_grp - 1) * _G
    W5 = 3 * NG * 50
    WOS = W5 + 3 * NG * _G
    WO5 = WOS + 49 * NG
    xres = stream.at[pl.ds(0, 2 * GR + S)]
    norm = stream.at[pl.ds(2 * GR + S, 2 * GR + S)]

    def half(h):
        return slice(h * HR, (h + 1) * HR)

    def of_group(ref, g, n=1):
        row = (g + 2) * GR
        return ref.at[pl.ds(row if isinstance(row, int) else pl.multiple_of(row, GR), n * GR)]

    def panel(ref, k, rows):
        return ref.at[rows, pl.ds(k * D if isinstance(k, int) else pl.multiple_of(k * D, _T), D)]

    def after_stores(ref):
        return ref.at[pl.ds(pl.multiple_of(zero_ref[0], 32), ref.shape[0])]

    def seg_operand(g, r, t, halves):
        rows = of_group(norm, g) if halves else None
        return [_lin2(_U, r, t, lambda i, k: rows[pl.ds(i * seg + h * HR, HR), _cols(k)])
                for h in halves]

    def lead_in(ns, ref, dst):
        todo = _merged(_VISITS[:3])
        lhs = {k: jnp.concatenate(seg_operand(0, *k, hs), axis=0) for k, hs in todo.items()}
        for n in ns:
            prods = {}
            for (r, t), hs in todo.items():
                res = _dot(lhs[r, t], _tiles(ref, n * 50 + r * 7 + t))
                prods.update({(r, t, h): res[half(u)] for u, h in enumerate(hs)})
            for (i, j, h), v in _add_blocks(_inner_blocks(prods, range(7)), _W, (), None).items():
                dst[n, i * _G + j, half(h), :] = v
            yield

    def finish_rows(g, first, n, update):
        rows = pl.ds(first, n)
        xn = of_group(xres, g)[rows, :] + jnp.concatenate(update, axis=1)
        of_group(xres, g)[rows, :] = xn
        of_group(norm, g)[rows, :] = _layernorm(_layernorm(xn), 0.5)

    def finish_stored(g, first, n):
        i, r0 = divmod(first, seg)
        finish_rows(g, first, n, [fin[i * (_G + 1) + j, r0:r0 + n, :] for j in range(_G + 1)])

    def step(layer, g, i, mem, side):
        last = side is not None
        early = layer == 0 and not last
        order = _Order(*(_LAST if last else _LEADING)[layer][i])
        final = last and i == _G - 1
        n_mem = 0 if final else M

        v_in = (i + 3) % 4
        p, q = _VISITS[v_in]

        def halves_in(r, t):
            return () if last and i else _halves(p, q, r, t)

        mem_lhs = _memory_operands(p, q, lambda k: mem[k])
        lhs = {k: jnp.concatenate(seg_operand(g + (i > 0), *k, halves_in(*k)) + [v], axis=0)
               for k, v in mem_lhs.items()}

        def last_tile_operand(src):
            return jnp.concatenate([of_group(src, g)[pl.ds(i * seg, seg), _cols(_G)], mem[_G]],
                                   axis=0)

        partial, kept = tbuf, cbuf
        if not last:
            z = (g + i) // (n_grp + _G)
            partial, kept = tbuf.at[pl.ds(z, 3 * NG)], cbuf.at[pl.ds(z, 3 * NG)]

        todo_in = _visit_order(order.in_outer, order.in_inner, order.in_turn, p, q)
        fifth = _digits(order.fifth)
        kqv = {}

        def project(n, lhs5):
            with_mem = not (final and n % 3 == 1)
            slot = n % 3 * NG + n // 3
            pre = HR if early and slot < _N_EARLY else 0
            lhs5 = lhs5[pre:] if with_mem else lhs5[:seg]
            mem_prods, prods, rest, inner, blocks = {}, {}, {}, {}, {}

            def last_tile(at):
                for j in range(_G):
                    if fifth[j] == at:
                        rest[j] = _dot(lhs5, _tiles(wt, W5 + n * _G + j))

            def combine(rs, outer_blocks):
                inner.update(_inner_blocks(prods, rs))
                new = _add_blocks(inner, outer_blocks, _VISITS[:v_in],
                                  lambda ii, j, h: partial[n, ii * _G + j, half(h), :])
                for (ii, j, h), v in new.items():
                    if i:
                        partial[n, ii * _G + j, half(h), :] = v
                    elif ii:
                        kept[n, (ii - 1) * _G + j, half(h), :] = v
                blocks.update(new)

            for pos, (r, ts) in enumerate(todo_in.items()):
                last_tile(2 * pos)
                if fifth[0] == 2 * pos:
                    yield
                for u, t in enumerate(ts):
                    if u == 2:
                        last_tile(2 * pos + 1)
                    if with_mem:
                        res = _dot(lhs[r, t], _tiles(wt, n * 50 + r * 7 + t))
                        hs = halves_in(r, t)
                        prods.update({(r, t, h): res[half(u)] for u, h in enumerate(hs)})
                        mem_prods[r, t] = res[len(hs) * HR:]
                if order.eager:
                    combine([r], [b for b in _W if r in _W[b]
                                  and not set(_W[b]) & set(list(todo_in)[pos + 1:])])
                if fifth[0] == 2 * pos + 1:
                    yield
                if pos < 3:
                    yield
            if not order.eager:
                combine(range(7), _W)
            if i:
                parts = [[kept[n, (i - 1) * _G + j]] for j in range(_G)]
            else:
                parts = [[blocks[0, j, 0], blocks[0, j, 1]] for j in range(_G)]
            if with_mem:
                parts = [a + [b] for a, b in zip(parts, _memory_result(p, q, mem_prods))]
            for j in range(_G):
                if pre:
                    src = _shifted(pool, g * _G * pre, (n_grp - 2) * _G * pre)
                    both = pltpu.bitcast(src[pl.ds((slot * n_lead + i) * pre, pre), _cols(j // 2)],
                                         _BF16).astype(_F32)
                    rest[j] = jnp.concatenate([both[half(j % 2)], rest[j]], axis=0)
                kqv[n, j] = jnp.concatenate(parts[j], axis=0) + rest[j]
            yield

        ri = lax.broadcasted_iota(jnp.int32, (seg, L), 0)
        ci = lax.broadcasted_iota(jnp.int32, (seg, L), 1)
        mask = (ci >= seg) | (ri >= ci)
        scale = _T ** -0.5
        o_new = obuf.at[pl.ds((g % 2) * _G, _G)]
        o_old = o_new if i == _G - 1 else obuf.at[pl.ds(((g + 1) % 2) * _G, _G)]
        o_mem, weights = {}, {}

        def score(gam, j):
            weights[gam, j] = _dot_nt(kqv.pop((3 * gam + 1, j)),
                                      kqv.pop((3 * gam, j)).astype(_BF16))

        def softmax(gam, j):
            sc = weights[gam, j]
            causal = jnp.where(mask, sc[:seg], -1e9 / scale)
            sc = causal if final else jnp.concatenate([causal, sc[seg:]], axis=0)
            e = jnp.exp2((sc - jnp.max(sc, axis=-1, keepdims=True)) * (scale * np.log2(np.e)))
            weights[gam, j] = e, pltpu.reciprocal(jnp.sum(e, axis=-1, keepdims=True), approx=True)

        def attend(gam, j):
            e, inv = weights.pop((gam, j))
            o = _dot(e, kqv.pop((3 * gam + 2, j)).astype(_BF16)) * inv
            o_new[i, :, _cols(gam * _G + j)] = o[:seg]
            o_mem[gam * _G + j] = [] if final else [o[seg:]]

        v_out = (i + 1) % 4
        po, qo = _VISITS[v_out]
        todo = _merged(_VISITS) if final else {
            (r, t): _halves(po, qo, r, t) for r, ts in _visit_order(
                order.out_outer, order.out_inner, order.out_turn, po, qo).items() for t in ts}
        acc = {}

        def out_main(g0, g1):
            riders = {} if final else {gam: _memory_operands(
                po, qo, lambda k: o_mem[gam * _G + k][0]) for gam in range(g0, g1)}
            for (r, t), hs in todo.items():
                a = jnp.concatenate([jnp.concatenate(
                    ([] if final else [riders[gam][r, t]])
                    + [_lin2(_U, r, t, lambda ii, k: o_old[ii, half(h), _cols(gam * _G + k)])
                       for h in hs], axis=0)
                    for gam in range(g0, g1)], axis=1)
                res = _dot(a, _tiles(wt, WOS + (r * 7 + t) * NG + g0, g1 - g0))
                acc[r, t] = res + acc[r, t] if (r, t) in acc else res

        def out_last(g0, g1):
            a = jnp.concatenate([jnp.concatenate(o_mem[hd] + [o_new[i, :, _cols(hd)]], axis=0)
                                 for hd in range(g0 * _G, g1 * _G)], axis=1)
            res = _dot(a, _tiles(wt, WO5 + g0 * _G, (g1 - g0) * _G))
            acc[-1] = res + acc[-1] if -1 in acc else res

        tasks = []
        for gam in range(NG):
            for j in range(_G):
                at = 5 * (3 * gam + 2) + order.score
                tasks += [(at, 1, score, gam, j),
                          (at + order.softmax, 1, softmax, gam, j),
                          (at + order.attend, 1, attend, gam, j)]
        for item in order.out_chunks.split():
            at, op = item.split(':')
            tasks.append((int(at), 0, out_main if op[0] == 'm' else out_last,
                          int(op[1]), int(op[2])))
        tasks.sort(key=lambda task: task[:2])
        now = 0
        lhs5 = last_tile_operand(norm)
        for n in range(3 * NG):
            if final:
                if 4 <= n < 4 + GR // 8:
                    finish_stored(g - 1, (n - 4) * 8, 8)
                    lhs5 = last_tile_operand(after_stores(norm))
            elif n in order.finish:
                finish_stored(g - 2 + (i == 3), v_out * seg + order.finish.index(n) * 8, 8)
                lhs5 = last_tile_operand(norm)
            if last and i in (1, 2) and n % 2:
                next(side, None)
                spare = (pl.ds(pool.shape[0] - M, M), _cols(0))
                pool[spare] = pltpu.bitcast(mem[_G], _U32)
                lhs5 = jnp.concatenate(
                    [lhs5[:seg], pltpu.bitcast(after_stores(pool)[spare], _F32)], axis=0)
            for _ in project(n, lhs5):
                now += 1
                while tasks and tasks[0][0] <= now:
                    _, _, f, a, b = tasks.pop(0)
                    f(a, b)
        for _, _, f, a, b in tasks:
            f(a, b)

        tail = acc.pop(-1)
        n5[g % 2, i * seg:(i + 1) * seg, :] = tail[n_mem:]
        prods = {(r, t, h): v[n_mem + u * HR:n_mem + (u + 1) * HR] for (r, t), v in acc.items()
                 for u, h in enumerate(todo[r, t])}
        blocks = _add_blocks(_inner_blocks(prods, range(7)), _W, () if final else _VISITS[:v_out],
                             lambda ii, j, h: mo[ii * _G + j, half(h), :])
        if final:
            for ii in range(_G):
                for h in (0, 1):
                    first = ii * seg + h * HR
                    finish_rows(g, first, HR, [blocks[ii, j, h] for j in range(_G)]
                                + [n5[g % 2, first:first + HR, :]])
            return None
        for (ii, j, h), v in blocks.items():
            if v_out == 3:
                fin[ii * (_G + 1) + j, half(h), :] = v
            else:
                mo[ii * _G + j, half(h), :] = v
        if v_out == 3:
            for ii in range(_G):
                fin[ii * (_G + 1) + _G] = n5[(g + 1) % 2, ii * seg:(ii + 1) * seg, :]
        return _memory_result(po, qo, {k: v[:M] for k, v in acc.items()}) + [tail[:M]]

    def group(layer, g, mem, side=None):
        for i in range(_G):
            mem = step(layer, g, i, mem, side)
        return mem

    def leading_groups(layer):
        mem0 = mem0_ref[0:M, :].astype(_F32)
        mem = lax.fori_loop(0, n_grp - 1, functools.partial(group, layer),
                            [mem0[:, _cols(k)] for k in range(_G + 1)])
        mem_ref[...] = jnp.concatenate(mem, axis=1)

    HD, QD = D // 2, D // _G
    NS = S // (_G * _T)
    NF = F // (_G * _T)
    F0 = _G * NF * _T

    def operand(r, t, c):
        return pl.ds((c // 2 * 49 + r * 7 + t) * QD, QD), _cols(c % 2)

    def token_operands(c, outer_order, inner_order):
        ht = [of_group(norm, _G * c + k)[...].T for k in range(_G)]
        for r in outer_order:
            outer = _outer(_U, r, lambda i, k: ht[k][i * QD:(i + 1) * QD])
            for t in inner_order:
                pool.bitcast(_BF16)[operand(r, t, c)] = _lin(_U[t], outer.get).astype(_BF16)
            yield

    def out_rows(blk, n):
        return panel(w1t, blk // (2 * _G), _cols(blk % (2 * _G), n))

    def out_copy(part):
        return pltpu.make_async_copy(out_rows(2 * part, 2), out_hbm.at[_cols(2 * part, 2)],
                                     sems.at[part])

    def mixer(layer):
        final = layer == 1
        outer1, inner1, outer2, inner2 = map(_digits, _MIXER[layer])
        ops = pool.bitcast(_BF16)
        b1 = jnp.concatenate([0.5 * b1_ref[...].astype(_F32).reshape(1, F),
                              jnp.zeros((1, F0 + 2 * _T - F), _F32)], axis=1)
        b2 = b2_ref[...].astype(_F32).reshape(1, S)
        hosts = {2: 1, 3: 0, 5: 1, 6: 0}

        def inner_blocks(r, order, dot, first, raw, n_k, axis, rest=None):
            outer = [_outer(_V, r, functools.partial(raw, kt)) for kt in range(n_k)]
            prods = {}
            for t in order:
                rhs = [_lin(_V[t], lambda n: o[_mirror(r, n)]) for o in outer]
                if rest and t in hosts:
                    rhs.append(rest[_mirror(r, (0, hosts[t]))[1]])
                a = jnp.concatenate([ops[operand(r, t, first + u)] for u in range(len(rhs))],
                                    axis=1)
                prods[t] = dot(a, jnp.concatenate(rhs, axis=axis).astype(_BF16))
            return {_mirror(r, n): _lin(coef, prods.get) for n, coef in _W.items()}

        def completed(r, inner):
            return [b for b, coef in _W.items() if r in coef and all(u in inner for u in coef)]

        u = None
        for c in range(NS):
            part = _dot(w1t[F0:F, _cols(_G * c, _G)], of_group(norm, _G * c, _G)[...].astype(_BF16))
            u = part if u is None else part + u
        u = jnp.concatenate([u, jnp.zeros((F0 + 2 * _T - F, D), _F32)], axis=0).T
        act = {(i, j): _gelu_of_twice(u[i * HD:(i + 1) * HD, _cols(j)] + b1[:, _cols(F0 // _T + j)])
               for i, j in _W}
        for r in range(7):
            outer = _lin(_U[r], act.get)
            for t in hosts:
                ops[operand(r, t, NS + NF)] = _lin(
                    _U[t], lambda n: outer[n[0] * QD:(n[0] + 1) * QD]).astype(_BF16)

        def hidden_operands(c, r, act):
            outer = _outer(_U, r, lambda i, k: act[i, k])
            for t in range(7):
                ops[operand(r, t, NS + c)] = _lin(_U[t], outer.get).astype(_BF16)

        list(token_operands(NS - 1, outer1, inner1))
        pending = []
        for c in range(NF):
            def raw1(kt, k, j):
                return w1t[_cols(j * NF + c), _cols(_G * kt + k)].astype(_F32)

            inner, act, queued = {}, {}, []
            for r in outer1:
                inner[r] = inner_blocks(r, inner1, _dot_nt, 0, raw1, NS, 1)
                for b in completed(r, inner):
                    for n in _W:
                        i, j = 2 * b[0] + n[0], 2 * b[1] + n[1]
                        act[i, j] = _gelu_of_twice(_lin(_W[b], lambda v: inner[v][n])
                                                   + b1[:, _cols(j * NF + c)])
                for v in outer2:
                    if v not in queued and all((2 * o[0], 2 * o[1]) in act for o in _U[v]):
                        queued.append(v)
                        pending.append((c, v, act))
                if pending:
                    hidden_operands(*pending.pop(0))
        for job in pending:
            hidden_operands(*job)

        def rest_rows(tile, c):
            lo = F0 + tile * _T
            w = w2n[lo:min(lo + _T, F), _cols(c)].astype(_F32)
            if lo + _T > F:
                w = jnp.concatenate([w, jnp.zeros((lo + _T - F, _T), _F32)], axis=0)
            return w

        for c in range(NS):
            def raw2(kt, k, j):
                w = w2n[_cols(k * NF + kt), _cols(_G * c + j)]
                if final and c and len(inner) == 1 and (kt, k, j) == (0, 0, 0):
                    spare = (slice(0, 16), _cols(S // _T - 1))
                    after_stores(w1t)[spare] = w[:16]
                    return jnp.concatenate([w1t[spare].astype(_F32), w[16:].astype(_F32)], axis=0)
                return w.astype(_F32)

            inner, done = {}, {}
            for r in outer2:
                rest = [_lin(_V[r], lambda kj: rest_rows(kj[0], _G * c + 2 * kj[1] + j2))
                        for j2 in (0, 1)]
                inner[r] = inner_blocks(r, inner2, _dot, NS, raw2, NF, 0, rest)
                if not final and c * 7 + len(inner) > 8:
                    next(next_layer)
                for b in completed(r, inner):
                    done[b] = {n: _lin(_W[b], lambda v: inner[v][n]) for n in _W}
                    if (1 - b[0], b[1]) not in done:
                        continue
                    for j2 in (0, 1):
                        blk = _G * c + 2 * b[1] + j2
                        y = jnp.concatenate([done[i // 2, b[1]][i % 2, j2] for i in range(_G)],
                                            axis=0)
                        xn = of_group(xres, blk)[...] + (y + b2[:, _cols(blk)]).T
                        if final:
                            out_rows(blk, 1)[...] = xn.astype(_BF16)
                        else:
                            of_group(xres, blk)[...] = xn
                            of_group(norm, blk)[...] = _layernorm(xn)
                    if final:
                        out_copy(2 * c + b[1]).start()

    def last_group(layer):
        side = (u for c in range(NS - 1)
                for u in token_operands(c, (2, 4, 6, 5, 1, 3, 0), _digits(_MIXER[layer][1])))
        group(layer, n_grp - 1, [mem_ref[:, _cols(k)] for k in range(_G + 1)], side)

    def stage():
        CR = _T // _CHUNKS
        per = NG // _CHUNKS
        WR = per * _G * _T

        def for_chunk(c, act):
            slot = c % _SLOTS
            which, part = (c + 1) // _CHUNKS, (c + 1) % _CHUNKS
            for m, w in enumerate((wk_hbm, wq_hbm, wv_hbm)):
                @pl.when(c == m)
                def _():
                    for k in range(_CHUNKS):
                        act(pltpu.make_async_copy(w.at[_G, pl.ds(k * CR * H, CR * H)],
                                                  ring.at[slot * _G + k, 0:CR * H],
                                                  sems.at[slot]))

                @pl.when(which == m + 1)
                def _():
                    act(pltpu.make_async_copy(w.at[pl.ds(0, _G), _aligned(part * CR * H, CR * H)],
                                              ring.at[pl.ds(slot * _G, _G), 0:CR * H],
                                              sems.at[slot]))

            @pl.when(which == 4)
            def _():
                act(pltpu.make_async_copy(wo_hbm.at[_aligned(part * WR, WR)],
                                          panel(w1t, slot, pl.ds(0, WR)), sems.at[slot]))

        def arrived(c):
            for_chunk(c, lambda cp: cp.wait())
            for_chunk(c + _SLOTS - 1, lambda cp: cp.start())
            return ring.at[pl.ds(c % _SLOTS * _G, _G)].bitcast(_U32)

        def head_group(words, k, u, gam):
            pairs = [words[k, pl.ds(u * 8 * H + gam * _G // 2 + a, 16, stride=H // 2), :]
                     for a in range(_G // 2)]
            return [pltpu.bitcast(bits, _F32)
                    for w in pairs for bits in (w << 16, w & np.uint32(0xFFFF0000))]

        pieces = 5

        def project_early(first, count):
            rows = n_lead // 2 * HR
            for k in [first + u for u in range(count)]:
                w = _shifted(wt, (k // 2 % NG * 3 + k // 2 // NG) * _T, (3 * NG - 1) * _T)
                src = early_lhs.at[_aligned(k % 2 * rows, rows)]
                dst = pool.at[_aligned(k * rows, rows)].bitcast(_BF16)
                for r0 in range(0, rows, rows // pieces):
                    res = _dot(src[r0:r0 + rows // pieces, :].astype(_BF16), _tiles(w, W5, _G, 1))
                    for s in range(0, rows // pieces, HR):
                        for jj in range(_G // 2):
                            dst[pl.ds(2 * (r0 + s), 2 * HR), _cols(jj)] = jnp.concatenate(
                                [res[s:s + HR, _cols(2 * jj + a)] for a in (0, 1)],
                                axis=0).astype(_BF16)
                    yield

        def combine_kqv(raw, m, c):
            dst = _shifted(wt, (m * 25 * _T + c * CR) // 2, 26 * _T).bitcast(_BF16)
            for u in range(CR // 16):
                for gam in range(NG):
                    heads = [head_group(raw, k, u, gam) for k in range(_G)]
                    for tile, v in _weight_tiles(lambda k, j: heads[k][j]):
                        _put_rows(dst, 3 * gam * 50 + tile, u * 16, v)
                    yield

        def combine_out(c):
            raw = panel(w1t, (3 + 3 * _CHUNKS + c) % _SLOTS, pl.ds(0, WR))
            dst = _shifted(wt, c * per * _T // 4, (_CHUNKS - 1) * per * _T // 4).bitcast(_BF16)
            dst5 = _shifted(wt, c * per * _T, (_CHUNKS - 1) * per * _T).bitcast(_BF16)
            for a in range(per):
                for u in range(_T // 16):
                    blocks = {(k, j): raw[pl.ds((a * _G + k) * _T + u * 16, 16), _cols(j)]
                              .astype(_F32) for k in range(_G) for j in range(_G + 1)}
                    for tile, v in _weight_tiles(lambda k, j: blocks[k, j]):
                        _put_rows(dst, WOS + tile * NG + a, u * 16, v)
                    for k in range(_G):
                        _put_rows(dst5, WO5 + a * _G + k, u * 16, blocks[k, _G])
                    yield

        def lead_in_part(m, c):
            n = 3 * per * c + m
            list(lead_in(range(0, 3 * per, 3),
                         _shifted(wt, n * 25 * _T // 2, (3 * NG - 4) * 25 * _T // 2),
                         tbuf.at[pl.ds(n, 3 * per - 2)]))

        def x_copy(c):
            n = S // _CHUNKS
            return pltpu.make_async_copy(x_hbm.at[_aligned(c * n, n)],
                                         panel(w2n, c // 2, _aligned(c % 2 * n, n)),
                                         sems.at[_SLOTS + c])

        mem_copy = pltpu.make_async_copy(mem0_hbm, mem0_ref.at[0:M], sems.at[_SLOTS + _CHUNKS])
        mem_copy.start()
        x_copy(0).start()
        x_copy(1).start()
        for ref in (fin, mo, n5):
            ref[...] = jnp.zeros_like(ref)
        xres[0:2 * GR, :] = jnp.zeros((2 * GR, D), _F32)
        for i in range(_G):
            obuf[_G + i] = jnp.zeros(obuf.shape[1:], _F32)
        mem_copy.wait()

        @pl.loop(0, _CHUNKS)
        def _(c):
            x_copy(c).wait()

            @pl.when(c + 2 < _CHUNKS)
            def _():
                x_copy(c + 2).start()

            @pl.when(c + 2 >= _CHUNKS)
            def _():
                for_chunk(c + 2 - _CHUNKS, lambda cp: cp.start())

            @pl.loop(c * (n_grp // _CHUNKS), (c + 1) * (n_grp // _CHUNKS))
            def _(g):
                x = panel(w2n, c // 2, _aligned(g % (n_grp // 2) * GR, GR))[...].astype(_F32)
                of_group(xres, g)[...] = x
                of_group(norm, g)[...] = _layernorm(x)

        for s in range(n_lead):
            early_lhs[half(s), :] = of_group(norm, s // _G)[pl.ds(s % _G * seg, HR), _cols(_G)]

        @pl.loop(0, 3)
        def _(m):
            raw = arrived(m)
            dst = _shifted(wt, m * _T, 2 * _T).bitcast(_BF16)
            for gam in range(NG):
                for k in range(_CHUNKS):
                    for u in range(CR // 16):
                        for j, v in enumerate(head_group(raw, k, u, gam)):
                            _put_rows(dst, W5 + 3 * gam * _G + j, k * CR + u * 16, v)
                if gam == 0:
                    list(project_early(m * _EARLY[0], _EARLY[0]))

        @pl.loop(0, _CHUNKS)
        def _(c):
            raw = arrived(3 + c)
            _interleave((combine_kqv(raw, 0, c), 16),
                        (project_early(3 * _EARLY[0] + c * _EARLY[1], _EARLY[1]),
                         _EARLY[1] * pieces))

        @pl.loop(0, 2 * _CHUNKS)
        def _(c):
            raw = arrived(3 + _CHUNKS + c)
            first = 3 * _EARLY[0] + _CHUNKS * _EARLY[1] + c * _EARLY[2]
            _interleave((combine_kqv(raw, c // _CHUNKS + 1, c % _CHUNKS), 16),
                        (project_early(first, _EARLY[2]), _EARLY[2] * pieces))
            lead_in_part(c // _CHUNKS, c % _CHUNKS)

        @pl.loop(0, _CHUNKS)
        def _(c):
            arrived(3 + 3 * _CHUNKS + c)
            first = 2 * _N_EARLY - (_CHUNKS - c) * _EARLY[3]
            _interleave((combine_out(c), 16), (project_early(first, _EARLY[3]), _EARLY[3] * pieces))
            lead_in_part(2, c)

    next_layer = lead_in(range(3 * NG), wt, tbuf)

    @pl.loop(0, zero_ref.shape[0])
    def _(u):
        zero_ref[u] = 0

    stage()
    mixer_copies = [pltpu.make_async_copy(src, dst, sems.at[u]) for u, (src, dst) in enumerate(
        ((w1_hbm, w1t), (w2_hbm, w2n), (b1_hbm, b1_ref), (b2_hbm, b2_ref)))]
    for cp in mixer_copies:
        cp.start()
    leading_groups(0)
    for cp in mixer_copies:
        cp.wait()
    last_group(0)
    mixer(0)
    list(next_layer)
    leading_groups(1)
    last_group(1)
    mixer(1)
    for part in range(2 * NS):
        out_copy(part).wait()


@functools.partial(jax.jit, static_argnames=("A_seg_len",))
def pallas_interleave_layers__memory_aug_recurrent_mem_tr__mixer_token_mlp__prompt_kernel(
    A_x: jax.Array,
    A_mem0: jax.Array,
    A_Wq: jax.Array,
    A_Wk: jax.Array,
    A_Wv: jax.Array,
    A_Wo: jax.Array,
    A_seg_len: int,
    B_x: jax.Array,
    B_w1: jax.Array,
    B_b1: jax.Array,
    B_w2: jax.Array,
    B_b2: jax.Array,
):
    del B_x
    _, S, D = A_x.shape
    _, H, E = A_Wq.shape
    M = A_mem0.shape[1]
    F = B_w1.shape[1]
    seg = int(A_seg_len)
    NG, GR = H // _G, _G * seg
    assert D == (_G + 1) * _T and E == _T and GR == _T
    hbm = pl.BlockSpec(memory_space=pl.ANY)
    by_tile = (_G + 1, _T * H, E)
    out = pl.pallas_call(
        functools.partial(_kernel, seg=seg),
        out_shape=jax.ShapeDtypeStruct((S, D), A_x.dtype),
        in_specs=[hbm] * 10,
        out_specs=hbm,
        scratch_shapes=[
            pltpu.VMEM((2 * (2 * GR + S), D), _F32),
            pltpu.VMEM((NG * (3 * 50 + 49 + 4 * _G) * _T // 4, 2 * _T), _U32),
            pltpu.VMEM((F, S), _BF16),
            pltpu.VMEM((F, S), _BF16),
            pltpu.VMEM((3 * NG, _G * _G, seg, _T), _F32),
            pltpu.VMEM((_G * _G, seg, _T), _F32),
            pltpu.VMEM((_G * (_G + 1), seg, _T), _F32),
            pltpu.VMEM((2, GR, _T), _F32),
            pltpu.VMEM((2 * _G, seg, H * E), _F32),
            pltpu.VMEM((_N_EARLY * (S - GR) // 2, 2 * _T), _U32),
            pltpu.VMEM((_SLOTS * _G, _T // _CHUNKS * H + 64, _T), _BF16),
            pltpu.VMEM((3 * NG, (_G - 1) * _G, seg, _T), _F32),
            pltpu.VMEM(((S - GR) // 2, _T), _F32),
            pltpu.VMEM((8 * M, D), A_mem0.dtype),
            pltpu.VMEM((M, D), _F32),
            pltpu.VMEM((F,), B_b1.dtype),
            pltpu.VMEM((S,), B_b2.dtype),
            pltpu.SMEM((2,), jnp.int32),
            pltpu.SemaphoreType.DMA((S // (2 * _T),)),
        ],
        compiler_params=pltpu.CompilerParams(vmem_limit_bytes=128 * 1024 * 1024),
        name="rmt_mixer",
    )(A_x.reshape(S, D), A_mem0.reshape(M, D), A_Wq.reshape(by_tile), A_Wk.reshape(by_tile),
      A_Wv.reshape(by_tile), A_Wo.reshape(H * E, D), B_w1.T, B_b1, B_w2, B_b2)
    return out.reshape(A_x.shape)
```
